```python
import jax
import jax.numpy as jnp

def _softmax(x, axis=-1):
    return jax.nn.softmax(x, axis=axis)
def _gelu(x):
    return jax.nn.gelu(x, approximate=True)
def _silu(x):
    return jax.nn.silu(x)
def _sigmoid(x):
    return jax.nn.sigmoid(x)
def _layernorm(x, axis=-1, eps=1e-5):
    m = jnp.mean(x, axis=axis, keepdims=True)
    v = jnp.var(x, axis=axis, keepdims=True)
    return (x - m) / jnp.sqrt(v + eps)
def _scatter_add(tgt, idx, src, axis=0):
    return tgt.at[idx].add(src)
def _segment_sum(src, seg, n):
    return jax.ops.segment_sum(src, seg, n)
class _Rng:
    def __init__(self, key):
        self._k = key
    def _next(self):
        self._k, sub = jax.random.split(self._k)
        return sub
    def normal(self, shape):
        return jax.random.normal(self._next(), shape, dtype=jnp.bfloat16)
    def randint(self, lo, hi, shape):
        return jax.random.randint(self._next(), shape, lo, hi, dtype=jnp.int32)
    def uniform(self, shape, lo=0.0, hi=1.0):
        return jax.random.uniform(self._next(), shape, jnp.bfloat16, lo, hi)
    def permutation(self, n):
        return jax.random.permutation(self._next(), n)


kernel_name = 'concat_heads__compressed_kv_cla__mha_block_cached__decode'

def setup_inputs():
    _rng = _Rng(jax.random.key(int.from_bytes(__import__("os").urandom(4), "little")))
    _w = (lambda a: (lambda t: t.astype(jnp.bfloat16) if jnp.issubdtype(t.dtype, jnp.floating) else t)(jnp.asarray(a)))
    def _A_setup():
        B, H, Sq, Sk, D, M = 4, 32, 1, 4096, 128, 512
        Dc = 4 * D
        return {
            "x": _w((lambda *s: _rng.normal(s) * 0.05)(B, Sq, M)),
            "c_kv": _w((lambda *s: _rng.normal(s) * 0.05)(B, Sk, Dc)),
            "w_q": _w((lambda *s: _rng.normal(s) * 0.05)(M, H, D) * (M ** -0.5)),
            "w_uk": _w((lambda *s: _rng.normal(s) * 0.05)(Dc, H, D) * (Dc ** -0.5)),
            "w_uv": _w((lambda *s: _rng.normal(s) * 0.05)(Dc, H, D) * (Dc ** -0.5)),
            "w_o": _w((lambda *s: _rng.normal(s) * 0.05)(H, D, M) * ((H * D) ** -0.5)),
        }
    _A_in = _A_setup()

    def _B_setup():
        B, Sq, D = 4, 1, 512
        H, Sk, Dh = 32, 4096, 128
        return {
            "x": _w((lambda *s: _rng.normal(s) * 0.05)(B, Sq, D)),
            "k_cache": _w((lambda *s: _rng.normal(s) * 0.05)(B, H, Sk, Dh)),
            "v_cache": _w((lambda *s: _rng.normal(s) * 0.05)(B, H, Sk, Dh)),
            "wq": _w((lambda *s: _rng.normal(s) * 0.05)(D, H * Dh) * (D ** -0.5)),
            "wo": _w((lambda *s: _rng.normal(s) * 0.05)(H * Dh, D) * ((H * Dh) ** -0.5)),
        }
    _B_in = _B_setup()

    return {
        "A_x": _A_in["x"],
        "A_c_kv": _A_in["c_kv"],
        "A_w_q": _A_in["w_q"],
        "A_w_uk": _A_in["w_uk"],
        "A_w_uv": _A_in["w_uv"],
        "A_w_o": _A_in["w_o"],
        "B_x": _B_in["x"],
        "B_k_cache": _B_in["k_cache"],
        "B_v_cache": _B_in["v_cache"],
        "B_wq": _B_in["wq"],
        "B_wo": _B_in["wo"],
    }

def reference(A_x, A_c_kv, A_w_q, A_w_uk, A_w_uv, A_w_o, B_x, B_k_cache, B_v_cache, B_wq, B_wo):
    def _A_ref(x, c_kv, w_q, w_uk, w_uv, w_o):
        B, Sq, M = x.shape[0], x.shape[1], x.shape[2]
        Sk = c_kv.shape[1]
        H, D = w_q.shape[1], w_q.shape[2]
        q = jnp.einsum("bqm,mhd->bhqd", x, w_q)
        k = jnp.einsum("bkc,chd->bhkd", c_kv, w_uk)
        v = jnp.einsum("bkc,chd->bhkd", c_kv, w_uv)
        scores = jnp.einsum("bhqd,bhkd->bhqk", q, k) * (D ** -0.5)
        off = Sk - Sq
        qi = jnp.arange(Sq)[:, None]
        kj = jnp.arange(Sk)[None, :]
        cmask = kj <= (qi + off)
        scores = jnp.where(cmask[None, None], scores, -1e9)
        p = _softmax(scores, axis=-1)
        ctx = jnp.einsum("bhqk,bhkd->bhqd", p, v)
        return jnp.einsum("bhqd,hdm->bqm", ctx, w_o)

    def _B_ref(x, k_cache, v_cache, wq, wo):
        B, Sq, D = x.shape
        H, Dh = 32, 128
        q = (lambda x, *d: x.transpose(*d))((x @ wq).reshape(B, Sq, H, Dh), 0, 2, 1, 3)
        scores = jnp.einsum("bhqd,bhkd->bhqk", q, k_cache) * (Dh ** -0.5)
        p = _softmax(scores, axis=-1)
        o = jnp.einsum("bhqk,bhkd->bhqd", p, v_cache)
        return (lambda x, *d: x.transpose(*d))(o, 0, 2, 1, 3).reshape(B, Sq, H * Dh) @ wo

    a = _A_ref(A_x, A_c_kv, A_w_q, A_w_uk, A_w_uv, A_w_o)
    b = _B_ref(B_x, B_k_cache, B_v_cache, B_wq, B_wo)
    return jnp.concatenate([a, b], axis=-1)
```

```python
import jax
import jax.numpy as jnp
from jax import lax
import jax.experimental.pallas as pl
import jax.experimental.pallas.tpu as pltpu

_B, _H, _SK, _D, _M, _DC = 4, 32, 4096, 128, 512, 512
_HG = 16
_NDESC = 32
_F32, _BF16 = jnp.float32, jnp.bfloat16
_NT = (((1,), (1,)), ((), ()))


def _dot(a, b):
    return jnp.dot(a, b, preferred_element_type=_F32)


def _dot_nt(a, b):
    return lax.dot_general(a, b, _NT, preferred_element_type=_F32)


def _iota(shape, dim):
    return lax.broadcasted_iota(jnp.int32, shape, dim)


def _kernel(ax_ref, ckv_hbm, awq_hbm, awuk_hbm, awuv_hbm, awo_hbm,
            bx_ref, k_hbm, v_hbm, bwq_hbm, bwo_hbm,
            out_ref,
            ckv_buf, awq_buf, awuk_buf, awuv_buf, awo_buf, bwq_buf, bwo_buf, kv_buf,
            e_ref, qb_ref, ob_ref, wsem, kvsem):
    scale = _D ** -0.5

    def issue(piece):
        def body(j, carry):
            for queue in range(2):
                src, dst, sem = piece(queue, j)
                pltpu.make_async_copy(src, dst, sem).start(priority=queue)
            return carry
        lax.fori_loop(0, _NDESC, body, 0)

    def rows(start, size):
        return pl.ds(pl.multiple_of(start, size), size)

    class Unit:
        def __init__(self, piece, whole, sem):
            self.start = lambda: issue(lambda queue, j: piece(queue, j) + (sem,))
            self.wait = lambda: pltpu.make_async_copy(whole, whole, sem).wait()

    def up_unit(hbm, buf, u, sem):
        def piece(queue, j):
            sl = rows(u * 256 + queue * 128 + j * 4, 4)
            return hbm.at[sl], buf.at[sl]
        return Unit(piece, buf.at[pl.ds(u * 256, 256)], sem)

    def bwq_unit(u, sem):
        def piece(queue, j):
            sl = (rows(u * 256 + queue * 128 + (j // 4) * 16, 16), rows((j % 4) * 1024, 1024))
            return bwq_hbm.at[sl], bwq_buf.at[sl]
        return Unit(piece, bwq_buf.at[pl.ds(u * 256, 256)], sem)

    def ckv_unit(b, u, sem):
        def piece(queue, j):
            sl = rows(u * 2048 + queue * 1024 + j * 32, 32)
            return ckv_hbm.at[b, sl], ckv_buf.at[b, sl]
        return Unit(piece, ckv_buf.at[b, pl.ds(u * 2048, 2048)], sem)

    def awo_unit(u, sem):
        def piece(queue, j):
            h, sl = u * 16 + queue * 8 + j // 4, rows((j % 4) * 32, 32)
            return awo_hbm.at[h, sl], awo_buf.at[h, sl]
        return Unit(piece, awo_buf.at[pl.ds(u * 16, 16)], sem)

    def bwo_unit(u, sem):
        def piece(queue, j):
            sl = rows(u * 2048 + queue * 1024 + j * 32, 32)
            return bwo_hbm.at[sl], bwo_buf.at[sl]
        return Unit(piece, bwo_buf.at[pl.ds(u * 2048, 2048)], sem)

    def kv_unit(pair, slot):
        b, h = pair // _H, pair % _H
        def piece(queue, j):
            sl = rows(j * 128, 128)
            return (k_hbm, v_hbm)[queue].at[b, h, sl], kv_buf.at[slot, queue, sl]
        return Unit(piece, kv_buf.at[slot], kvsem.at[slot])

    def head_diag(t):
        keep = (_iota(t.shape, 0) & (_HG - 1)) == (_iota(t.shape, 1) & (_HG - 1))
        return jnp.where(keep, t, 0.0).astype(_BF16)

    def spread(x):
        return head_diag(_dot(x, e_ref[...]))

    def slab(buf, c, g):
        w = buf[c * 128:(c + 1) * 128, g * _HG:(g + 1) * _HG, :]
        return w.reshape(128 * _HG, _D)

    def softmax_parts(s):
        p = jnp.exp(s - jnp.max(s, axis=-1, keepdims=True))
        return p.astype(_BF16), jnp.sum(p, axis=-1, keepdims=True)

    st = {}

    def setup():
        e_ref[...] = ((_iota(e_ref.shape, 1) // _HG) == _iota(e_ref.shape, 0)).astype(_BF16)
        ob_ref[...] = jnp.zeros(ob_ref.shape, _F32)

    def b_query():
        row = _iota((8, _M), 0)
        x = jnp.zeros((8, _M), _F32)
        for b in range(_B):
            x = jnp.where(row == b, bx_ref[b].astype(_F32), x)
        q = _dot(x.astype(_BF16), bwq_buf[...])
        for h in range(_H):
            qb_ref[h] = q[:, h * _D:(h + 1) * _D]

    def a_query(u):
        if u == 0:
            st["x"] = jnp.concatenate(
                [jnp.broadcast_to(ax_ref[b].astype(_F32), (_HG, _M)) for b in range(_B)],
                axis=0).astype(_BF16)
            st["q"] = [jnp.zeros((_B * _HG, _D), _F32)] * 2
        for c in (2 * u, 2 * u + 1):
            lhs = spread(st["x"][:, c * 128:(c + 1) * 128])
            st["q"] = [st["q"][g] + _dot(lhs, slab(awq_buf, c, g)) for g in range(2)]

    def a_absorb(u):
        if u == 0:
            st["qabs"] = [[], []]
        for c in (2 * u, 2 * u + 1):
            for g in range(2):
                t = head_diag(_dot_nt(st["q"][g].astype(_BF16), slab(awuk_buf, c, g)))
                st["qabs"][g].append(_dot_nt(t, e_ref[...]).astype(_BF16))

    def a_scores(b, u):
        if u == 0:
            st["qb"] = jnp.concatenate(
                [jnp.concatenate([t[b * _HG:(b + 1) * _HG] for t in st["qabs"][g]], axis=1)
                 for g in range(2)], axis=0)
        c = ckv_buf[b, u * 2048:(u + 1) * 2048, :]
        s = _dot_nt(st["qb"], c) * scale
        m = jnp.max(s, axis=-1, keepdims=True)
        if u == 0:
            p = jnp.exp(s - m)
            st["m"], st["l"] = m, jnp.sum(p, axis=-1, keepdims=True)
            st["acc"] = _dot(p.astype(_BF16), c)
        else:
            m = jnp.maximum(m, st["m"])
            alpha = jnp.exp(st["m"] - m)
            p = jnp.exp(s - m)
            l = alpha * st["l"] + jnp.sum(p, axis=-1, keepdims=True)
            acc = alpha * st["acc"] + _dot(p.astype(_BF16), c)
            st.setdefault("lat", []).append((acc / l).astype(_BF16))

    def a_context(u):
        if u == 0:
            st["latg"] = [jnp.concatenate([t[g * _HG:(g + 1) * _HG] for t in st["lat"]], axis=0)
                          for g in range(2)]
            st["ctx"] = [jnp.zeros((_B * _HG, _D), _F32)] * 2
        for c in (2 * u, 2 * u + 1):
            st["ctx"] = [st["ctx"][g] + _dot(spread(st["latg"][g][:, c * 128:(c + 1) * 128]),
                                             slab(awuv_buf, c, g)) for g in range(2)]

    def a_out(g):
        shape = (_HG * 8, _B * _HG)
        r, c = _iota(shape, 0), _iota(shape, 1)
        perm = (((r & 7) * _HG + (r >> 3)) == c).astype(_BF16)
        t = _dot(perm, st["ctx"][g].astype(_BF16))
        lhs = jnp.concatenate([t[h * 8:(h + 1) * 8] for h in range(_HG)], axis=1)
        w = awo_buf[g * _HG:(g + 1) * _HG].reshape(_HG * _D, _M)
        o = _dot(lhs.astype(_BF16), w)
        st["oa"] = o if g == 0 else st["oa"] + o
        if g == 1:
            for b in range(_B):
                out_ref[b, :, 0:_M] = st["oa"][b:b + 1].astype(out_ref.dtype)

    def b_attend(pair, slot):
        b, h = pair // _H, pair % _H
        s = _dot_nt(qb_ref[h].astype(_BF16), kv_buf[slot, 0]) * scale
        p, l = softmax_parts(s)
        o = _dot(p, kv_buf[slot, 1]) / l
        ob_ref[h] = jnp.where(_iota(o.shape, 0) == b, o, ob_ref[h])

    def b_out(g):
        lhs = jnp.concatenate([ob_ref[g * _HG + h] for h in range(_HG)], axis=1)
        o = _dot(lhs.astype(_BF16), bwo_buf[g * 2048:(g + 1) * 2048, :])
        st["ob"] = o if g == 0 else st["ob"] + o
        if g == 1:
            for b in range(_B):
                out_ref[b, :, _M:2 * _M] = st["ob"][b:b + 1].astype(out_ref.dtype)

    head = []
    def add(make, compute):
        head.append((make(wsem.at[len(head)]), compute))

    for u in range(2):
        add(lambda s: bwq_unit(u, s), b_query if u == 1 else None)
    for u in range(2):
        add(lambda s: up_unit(awq_hbm, awq_buf, u, s), lambda u=u: a_query(u))
    for u in range(2):
        add(lambda s: up_unit(awuk_hbm, awuk_buf, u, s), lambda u=u: a_absorb(u))
    for b in range(_B):
        for u in range(2):
            add(lambda s: ckv_unit(b, u, s), lambda b=b, u=u: a_scores(b, u))
    for u in range(2):
        add(lambda s: up_unit(awuv_hbm, awuv_buf, u, s), lambda u=u: a_context(u))
    for u in range(2):
        add(lambda s: awo_unit(u, s), lambda u=u: a_out(u))
    n_head, n_pair = len(head), _B * _H
    tail = [bwo_unit(u, wsem.at[n_head + u]) for u in range(2)]

    head[0][0].start()
    head[1][0].start()
    setup()
    for i, (unit, compute) in enumerate(head):
        unit.wait()
        if compute is not None:
            compute()
        if i + 2 < n_head:
            head[i + 2][0].start()
        else:
            kv_unit(i + 2 - n_head, i + 2 - n_head).start()

    def pair_step(pair, carry):
        slot = pair % 2
        kv_unit(pair, slot).wait()
        b_attend(pair, slot)

        @pl.when(pair + 2 < n_pair)
        def _():
            kv_unit(pair + 2, slot).start()

        for u in range(2):
            @pl.when(pair + 2 == n_pair + u)
            def _():
                tail[u].start()
        return carry

    lax.fori_loop(0, n_pair, pair_step, 0)

    for u in range(2):
        tail[u].wait()
        b_out(u)


@jax.jit
def pallas_concat_heads__compressed_kv_cla__mha_block_cached__decode_kernel(
    A_x: jax.Array,
    A_c_kv: jax.Array,
    A_w_q: jax.Array,
    A_w_uk: jax.Array,
    A_w_uv: jax.Array,
    A_w_o: jax.Array,
    B_x: jax.Array,
    B_k_cache: jax.Array,
    B_v_cache: jax.Array,
    B_wq: jax.Array,
    B_wo: jax.Array,
):
    assert A_x.shape == (_B, 1, _M) and A_c_kv.shape == (_B, _SK, _DC)
    assert A_w_q.shape == (_M, _H, _D) and B_k_cache.shape == (_B, _H, _SK, _D)

    hbm = pl.BlockSpec(memory_space=pl.ANY)
    vmem = pl.BlockSpec(memory_space=pltpu.VMEM)
    return pl.pallas_call(
        _kernel,
        in_specs=[vmem, hbm, hbm, hbm, hbm, hbm, vmem, hbm, hbm, hbm, hbm],
        out_specs=vmem,
        out_shape=jax.ShapeDtypeStruct((_B, 1, 2 * _M), A_x.dtype),
        scratch_shapes=[
            pltpu.VMEM(A_c_kv.shape, _BF16),
            pltpu.VMEM(A_w_q.shape, _BF16),
            pltpu.VMEM(A_w_uk.shape, _BF16),
            pltpu.VMEM(A_w_uv.shape, _BF16),
            pltpu.VMEM(A_w_o.shape, _BF16),
            pltpu.VMEM(B_wq.shape, _BF16),
            pltpu.VMEM(B_wo.shape, _BF16),
            pltpu.VMEM((2, 2, _SK, _D), _BF16),
            pltpu.VMEM((128, 128 * _HG), _BF16),
            pltpu.VMEM((_H, 8, _D), _F32),
            pltpu.VMEM((_H, 8, _D), _F32),
            pltpu.SemaphoreType.DMA((20,)),
            pltpu.SemaphoreType.DMA((2,)),
        ],
        compiler_params=pltpu.CompilerParams(vmem_limit_bytes=96 * 1024 * 1024),
    )(A_x, A_c_kv, A_w_q, A_w_uk, A_w_uv, A_w_o, B_x, B_k_cache, B_v_cache, B_wq, B_wo)
```

```python
import jax
import jax.numpy as jnp
from jax import lax
import jax.experimental.pallas as pl
import jax.experimental.pallas.tpu as pltpu

_B, _H, _SK, _D, _M, _DC = 4, 32, 4096, 128, 512, 512
_HG = 16
_NDESC = 32
_AHEAD = 3
_F32, _BF16 = jnp.float32, jnp.bfloat16
_NT = (((1,), (1,)), ((), ()))


def _dot(a, b):
    return jnp.dot(a, b, preferred_element_type=_F32)


def _dot_nt(a, b):
    return lax.dot_general(a, b, _NT, preferred_element_type=_F32)


def _iota(shape, dim):
    return lax.broadcasted_iota(jnp.int32, shape, dim)


def _kernel(ax_ref, ckv_hbm, awq_hbm, awuk_hbm, awuv_hbm, awo_hbm,
            bx_ref, k_hbm, v_hbm, bwq_hbm, bwo_hbm,
            out_ref,
            ckv_buf, awq_buf, awuk_buf, awuv_buf, awo_buf, bwq_buf, bwo_buf, kv_buf,
            e_ref, qb_ref, ob_ref, part_ref, wsem, kvsem):
    scale = _D ** -0.5

    def issue(piece):
        def body(j, carry):
            for queue in range(2):
                src, dst, sem = piece(queue, j)
                pltpu.make_async_copy(src, dst, sem).start(priority=queue)
            return carry
        lax.fori_loop(0, _NDESC, body, 0)

    def rows(start, size):
        return pl.ds(pl.multiple_of(start, size), size)

    class Unit:
        def __init__(self, piece, whole, sem):
            self.start = lambda: issue(lambda queue, j: piece(queue, j) + (sem,))
            self.wait = lambda: pltpu.make_async_copy(whole, whole, sem).wait()

    def up_unit(hbm, buf, u, sem):
        def piece(queue, j):
            sl = rows(u * 256 + queue * 128 + j * 4, 4)
            return hbm.at[sl], buf.at[sl]
        return Unit(piece, buf.at[pl.ds(u * 256, 256)], sem)

    def bwq_unit(u, sem):
        def piece(queue, j):
            sl = (rows(u * 256 + queue * 128 + (j // 4) * 16, 16), rows((j % 4) * 1024, 1024))
            return bwq_hbm.at[sl], bwq_buf.at[sl]
        return Unit(piece, bwq_buf.at[pl.ds(u * 256, 256)], sem)

    def ckv_unit(b, u, sem):
        def piece(queue, j):
            sl = rows(u * 2048 + queue * 1024 + j * 32, 32)
            return ckv_hbm.at[b, sl], ckv_buf.at[b, sl]
        return Unit(piece, ckv_buf.at[b, pl.ds(u * 2048, 2048)], sem)

    def awo_unit(u, sem):
        def piece(queue, j):
            h, sl = u * 16 + queue * 8 + j // 4, rows((j % 4) * 32, 32)
            return awo_hbm.at[h, sl], awo_buf.at[h, sl]
        return Unit(piece, awo_buf.at[pl.ds(u * 16, 16)], sem)

    def bwo_unit(u, sem):
        def piece(queue, j):
            sl = rows(u * 2048 + queue * 1024 + j * 32, 32)
            return bwo_hbm.at[sl], bwo_buf.at[sl]
        return Unit(piece, bwo_buf.at[pl.ds(u * 2048, 2048)], sem)

    def kv_unit(pair, slot):
        b, h = pair // _H, pair % _H
        def piece(queue, j):
            sl = rows(j * 128, 128)
            return (k_hbm, v_hbm)[queue].at[b, h, sl], kv_buf.at[slot, queue, sl]
        return Unit(piece, kv_buf.at[slot], kvsem.at[slot])

    def head_diag(t):
        keep = (_iota(t.shape, 0) & (_HG - 1)) == (_iota(t.shape, 1) & (_HG - 1))
        return jnp.where(keep, t, 0.0).astype(_BF16)

    def spread(x):
        return head_diag(_dot(x, e_ref[...]))

    def slab(buf, c, g):
        w = buf[c * 128:(c + 1) * 128, g * _HG:(g + 1) * _HG, :]
        return w.reshape(128 * _HG, _D)

    def softmax_parts(s):
        p = jnp.exp(s - jnp.max(s, axis=-1, keepdims=True))
        return p.astype(_BF16), jnp.sum(p, axis=-1, keepdims=True)

    st = {}

    def setup():
        e_ref[...] = ((_iota(e_ref.shape, 1) // _HG) == _iota(e_ref.shape, 0)).astype(_BF16)
        ob_ref[...] = jnp.zeros(ob_ref.shape, _F32)

    def b_query():
        row = _iota((8, _M), 0)
        bx = bx_ref[...].astype(_F32)
        x = jnp.zeros((8, _M), _F32)
        for b in range(_B):
            x = jnp.where(row == b, bx[b:b + 1], x)
        q = _dot(x.astype(_BF16), bwq_buf[...])
        for h in range(_H):
            qb_ref[h] = q[:, h * _D:(h + 1) * _D]

    def a_query(u):
        if u == 0:
            ax = ax_ref[...].astype(_F32)
            st["x"] = jnp.concatenate(
                [jnp.broadcast_to(ax[b:b + 1], (_HG, _M)) for b in range(_B)],
                axis=0).astype(_BF16)
            st["q"] = [jnp.zeros((_B * _HG, _D), _F32)] * 2
        for c in (2 * u, 2 * u + 1):
            lhs = spread(st["x"][:, c * 128:(c + 1) * 128])
            st["q"] = [st["q"][g] + _dot(lhs, slab(awq_buf, c, g)) for g in range(2)]

    def a_absorb(u):
        if u == 0:
            st["qabs"] = [[], []]
        for c in (2 * u, 2 * u + 1):
            for g in range(2):
                t = head_diag(_dot_nt(st["q"][g].astype(_BF16), slab(awuk_buf, c, g)))
                st["qabs"][g].append(_dot_nt(t, e_ref[...]).astype(_BF16))

    def a_scores(b, u):
        if u == 0:
            st["qb"] = jnp.concatenate(
                [jnp.concatenate([t[b * _HG:(b + 1) * _HG] for t in st["qabs"][g]], axis=1)
                 for g in range(2)], axis=0)
        c = ckv_buf[b, u * 2048:(u + 1) * 2048, :]
        s = _dot_nt(st["qb"], c) * scale
        m = jnp.max(s, axis=-1, keepdims=True)
        if u == 0:
            p = jnp.exp(s - m)
            st["m"], st["l"] = m, jnp.sum(p, axis=-1, keepdims=True)
            st["acc"] = _dot(p.astype(_BF16), c)
        else:
            m = jnp.maximum(m, st["m"])
            alpha = jnp.exp(st["m"] - m)
            p = jnp.exp(s - m)
            l = alpha * st["l"] + jnp.sum(p, axis=-1, keepdims=True)
            acc = alpha * st["acc"] + _dot(p.astype(_BF16), c)
            st.setdefault("lat", []).append((acc / l).astype(_BF16))

    def a_context(u):
        if u == 0:
            st["latg"] = [jnp.concatenate([t[g * _HG:(g + 1) * _HG] for t in st["lat"]], axis=0)
                          for g in range(2)]
            st["ctx"] = [jnp.zeros((_B * _HG, _D), _F32)] * 2
        for c in (2 * u, 2 * u + 1):
            st["ctx"] = [st["ctx"][g] + _dot(spread(st["latg"][g][:, c * 128:(c + 1) * 128]),
                                             slab(awuv_buf, c, g)) for g in range(2)]

    def a_out(g):
        shape = (_HG * 8, _B * _HG)
        r, c = _iota(shape, 0), _iota(shape, 1)
        perm = (((r & 7) * _HG + (r >> 3)) == c).astype(_BF16)
        t = _dot(perm, st["ctx"][g].astype(_BF16))
        lhs = jnp.concatenate([t[h * 8:(h + 1) * 8] for h in range(_HG)], axis=1)
        w = awo_buf[g * _HG:(g + 1) * _HG].reshape(_HG * _D, _M)
        o = _dot(lhs.astype(_BF16), w)
        if g == 0:
            part_ref[...] = o
        else:
            out_ref[:, 0:_M] = (part_ref[...] + o)[0:_B].astype(out_ref.dtype)

    def b_attend(pair, slot):
        b, h = pair // _H, pair % _H
        s = _dot_nt(qb_ref[h].astype(_BF16), kv_buf[slot, 0]) * scale
        p, l = softmax_parts(s)
        o = _dot(p, kv_buf[slot, 1]) / l
        ob_ref[h] = jnp.where(_iota(o.shape, 0) == b, o, ob_ref[h])

    def b_out(g):
        lhs = jnp.concatenate([ob_ref[g * _HG + h] for h in range(_HG)], axis=1)
        o = _dot(lhs.astype(_BF16), bwo_buf[g * 2048:(g + 1) * 2048, :])
        if g == 0:
            part_ref[...] = o
        else:
            out_ref[:, _M:2 * _M] = (part_ref[...] + o)[0:_B].astype(out_ref.dtype)

    head = []
    def add(make, compute):
        head.append((make(wsem.at[len(head)]), compute))

    for u in range(2):
        add(lambda s: bwq_unit(u, s), b_query if u == 1 else None)
    for u in range(2):
        add(lambda s: up_unit(awq_hbm, awq_buf, u, s), lambda u=u: a_query(u))
    for u in range(2):
        add(lambda s: up_unit(awuk_hbm, awuk_buf, u, s), lambda u=u: a_absorb(u))
    for b in range(_B):
        for u in range(2):
            add(lambda s: ckv_unit(b, u, s), lambda b=b, u=u: a_scores(b, u))
    for u in range(2):
        add(lambda s: up_unit(awuv_hbm, awuv_buf, u, s), lambda u=u: a_context(u))
    for u in range(2):
        add(lambda s: awo_unit(u, s), lambda u=u: a_out(u))
    n_head, n_pair = len(head), _B * _H
    tail = [bwo_unit(u, wsem.at[n_head + u]) for u in range(2)]

    for i in range(_AHEAD):
        head[i][0].start()
    setup()
    for i, (unit, compute) in enumerate(head):
        unit.wait()
        if compute is not None:
            compute()
        if i + _AHEAD < n_head:
            head[i + _AHEAD][0].start()
        else:
            kv_unit(i + _AHEAD - n_head, i + _AHEAD - n_head).start()

    def pair_step(pair, carry):
        slot = pair % _AHEAD
        kv_unit(pair, slot).wait()
        b_attend(pair, slot)

        @pl.when(pair + _AHEAD < n_pair)
        def _():
            kv_unit(pair + _AHEAD, slot).start()

        for u in range(2):
            @pl.when(pair + _AHEAD == n_pair + u)
            def _():
                tail[u].start()
        return carry

    lax.fori_loop(0, n_pair, pair_step, 0)

    for u in range(2):
        tail[u].wait()
        b_out(u)


@jax.jit
def pallas_concat_heads__compressed_kv_cla__mha_block_cached__decode_kernel(
    A_x: jax.Array,
    A_c_kv: jax.Array,
    A_w_q: jax.Array,
    A_w_uk: jax.Array,
    A_w_uv: jax.Array,
    A_w_o: jax.Array,
    B_x: jax.Array,
    B_k_cache: jax.Array,
    B_v_cache: jax.Array,
    B_wq: jax.Array,
    B_wo: jax.Array,
):
    assert A_x.shape == (_B, 1, _M) and A_c_kv.shape == (_B, _SK, _DC)
    assert A_w_q.shape == (_M, _H, _D) and B_k_cache.shape == (_B, _H, _SK, _D)

    hbm = pl.BlockSpec(memory_space=pl.ANY)
    vmem = pl.BlockSpec(memory_space=pltpu.VMEM)
    out = pl.pallas_call(
        _kernel,
        in_specs=[vmem, hbm, hbm, hbm, hbm, hbm, vmem, hbm, hbm, hbm, hbm],
        out_specs=vmem,
        out_shape=jax.ShapeDtypeStruct((_B, 2 * _M), A_x.dtype),
        scratch_shapes=[
            pltpu.VMEM(A_c_kv.shape, _BF16),
            pltpu.VMEM(A_w_q.shape, _BF16),
            pltpu.VMEM(A_w_uk.shape, _BF16),
            pltpu.VMEM(A_w_uv.shape, _BF16),
            pltpu.VMEM(A_w_o.shape, _BF16),
            pltpu.VMEM(B_wq.shape, _BF16),
            pltpu.VMEM(B_wo.shape, _BF16),
            pltpu.VMEM((_AHEAD, 2, _SK, _D), _BF16),
            pltpu.VMEM((128, 128 * _HG), _BF16),
            pltpu.VMEM((_H, 8, _D), _F32),
            pltpu.VMEM((_H, 8, _D), _F32),
            pltpu.VMEM((8, _M), _F32),
            pltpu.SemaphoreType.DMA((20,)),
            pltpu.SemaphoreType.DMA((_AHEAD,)),
        ],
        compiler_params=pltpu.CompilerParams(vmem_limit_bytes=96 * 1024 * 1024),
    )(A_x.reshape(_B, _M), A_c_kv, A_w_q, A_w_uk, A_w_uv, A_w_o,
      B_x.reshape(_B, _M), B_k_cache, B_v_cache, B_wq, B_wo)
    return out.reshape(_B, 1, 2 * _M)
```

```python
import jax
import jax.numpy as jnp
from jax import lax
import jax.experimental.pallas as pl
import jax.experimental.pallas.tpu as pltpu

_B, _H, _SK, _D, _M, _DC = 4, 32, 4096, 128, 512, 512
_HG = 16
_NDESC = 32
_AHEAD = 3
_TAIL = ((0, 16), (16, 8), (24, 4), (28, 2), (30, 1), (31, 1))
_F32, _BF16 = jnp.float32, jnp.bfloat16
_NT = (((1,), (1,)), ((), ()))


def _dot(a, b):
    return jnp.dot(a, b, preferred_element_type=_F32)


def _dot_nt(a, b):
    return lax.dot_general(a, b, _NT, preferred_element_type=_F32)


def _iota(shape, dim):
    return lax.broadcasted_iota(jnp.int32, shape, dim)


def _kernel(ax_hbm, ckv_hbm, awq_hbm, awuk_hbm, awuv_hbm, awo_hbm,
            bx_hbm, k_hbm, v_hbm, bwq_hbm, bwo_hbm,
            out_ref,
            ax_ref, bx_ref,
            ckv_buf, awq_buf, awuk_buf, awuv_buf, awo_buf, bwq_buf, bwo_buf, kv_buf,
            e_ref, qb_ref, ob_ref, part_ref, xsem, wsem, kvsem):
    scale = _D ** -0.5

    def issue(piece, count):
        def body(j, carry):
            for queue in range(2):
                src, dst, sem = piece(queue, j)
                pltpu.make_async_copy(src, dst, sem).start(priority=queue)
            return carry
        lax.fori_loop(0, count, body, 0)

    def rows(start, size):
        return pl.ds(pl.multiple_of(start, size), size)

    class Unit:
        def __init__(self, piece, whole, sem, count=_NDESC):
            self.start = lambda: issue(lambda queue, j: piece(queue, j) + (sem,), count)
            self.wait = lambda: pltpu.make_async_copy(whole, whole, sem).wait()

    def up_unit(hbm, buf, u, sem):
        def piece(queue, j):
            sl = rows(u * 256 + queue * 128 + j * 4, 4)
            return hbm.at[sl], buf.at[sl]
        return Unit(piece, buf.at[pl.ds(u * 256, 256)], sem)

    def bwq_unit(u, sem):
        def piece(queue, j):
            sl = (rows(u * 256 + queue * 128 + (j // 4) * 16, 16), rows((j % 4) * 1024, 1024))
            return bwq_hbm.at[sl], bwq_buf.at[sl]
        return Unit(piece, bwq_buf.at[pl.ds(u * 256, 256)], sem)

    def ckv_unit(b, u, sem):
        def piece(queue, j):
            sl = rows(u * 2048 + queue * 1024 + j * 32, 32)
            return ckv_hbm.at[b, sl], ckv_buf.at[b, sl]
        return Unit(piece, ckv_buf.at[b, pl.ds(u * 2048, 2048)], sem)

    def awo_unit(u, sem):
        def piece(queue, j):
            h, sl = u * 16 + queue * 8 + j // 4, rows((j % 4) * 32, 32)
            return awo_hbm.at[h, sl], awo_buf.at[h, sl]
        return Unit(piece, awo_buf.at[pl.ds(u * 16, 16)], sem)

    def bwo_unit(h0, nh, sem):
        def piece(queue, j):
            sl = rows(h0 * _D + queue * nh * (_D // 2) + j * 32, 32)
            return bwo_hbm.at[sl], bwo_buf.at[sl]
        return Unit(piece, bwo_buf.at[pl.ds(h0 * _D, nh * _D)], sem, count=2 * nh)

    def kv_unit(pair, slot):
        b, h = pair // _H, pair % _H
        def piece(queue, j):
            sl = rows(j * 128, 128)
            return (k_hbm, v_hbm)[queue].at[b, h, sl], kv_buf.at[slot, queue, sl]
        return Unit(piece, kv_buf.at[slot], kvsem.at[slot])

    def head_diag(t):
        keep = (_iota(t.shape, 0) & (_HG - 1)) == (_iota(t.shape, 1) & (_HG - 1))
        return jnp.where(keep, t, 0.0).astype(_BF16)

    def spread(x):
        return head_diag(_dot(x, e_ref[...]))

    def slab(buf, c, g):
        w = buf[c * 128:(c + 1) * 128, g * _HG:(g + 1) * _HG, :]
        return w.reshape(128 * _HG, _D)

    def softmax_parts(s):
        p = jnp.exp(s - jnp.max(s, axis=-1, keepdims=True))
        return p.astype(_BF16), jnp.sum(p, axis=-1, keepdims=True)

    st = {}

    def setup():
        e_ref[...] = ((_iota(e_ref.shape, 1) // _HG) == _iota(e_ref.shape, 0)).astype(_BF16)
        ob_ref[...] = jnp.zeros(ob_ref.shape, _F32)

    def b_query():
        row = _iota((8, _M), 0)
        bx = bx_ref[...].astype(_F32)
        x = jnp.zeros((8, _M), _F32)
        for b in range(_B):
            x = jnp.where(row == b, bx[b:b + 1], x)
        q = _dot(x.astype(_BF16), bwq_buf[...])
        for h in range(_H):
            qb_ref[h] = q[:, h * _D:(h + 1) * _D]

    def a_query(u):
        if u == 0:
            ax = ax_ref[...].astype(_F32)
            st["x"] = jnp.concatenate(
                [jnp.broadcast_to(ax[b:b + 1], (_HG, _M)) for b in range(_B)],
                axis=0).astype(_BF16)
            st["q"] = [jnp.zeros((_B * _HG, _D), _F32)] * 2
        for c in (2 * u, 2 * u + 1):
            lhs = spread(st["x"][:, c * 128:(c + 1) * 128])
            st["q"] = [st["q"][g] + _dot(lhs, slab(awq_buf, c, g)) for g in range(2)]

    def a_absorb(u):
        if u == 0:
            st["qabs"] = [[], []]
        for c in (2 * u, 2 * u + 1):
            for g in range(2):
                t = head_diag(_dot_nt(st["q"][g].astype(_BF16), slab(awuk_buf, c, g)))
                st["qabs"][g].append(_dot_nt(t, e_ref[...]).astype(_BF16))

    def a_scores(b, u):
        if u == 0:
            st["qb"] = jnp.concatenate(
                [jnp.concatenate([t[b * _HG:(b + 1) * _HG] for t in st["qabs"][g]], axis=1)
                 for g in range(2)], axis=0)
        c = ckv_buf[b, u * 2048:(u + 1) * 2048, :]
        s = _dot_nt(st["qb"], c) * scale
        m = jnp.max(s, axis=-1, keepdims=True)
        if u == 0:
            p = jnp.exp(s - m)
            st["m"], st["l"] = m, jnp.sum(p, axis=-1, keepdims=True)
            st["acc"] = _dot(p.astype(_BF16), c)
        else:
            m = jnp.maximum(m, st["m"])
            alpha = jnp.exp(st["m"] - m)
            p = jnp.exp(s - m)
            l = alpha * st["l"] + jnp.sum(p, axis=-1, keepdims=True)
            acc = alpha * st["acc"] + _dot(p.astype(_BF16), c)
            st.setdefault("lat", []).append((acc / l).astype(_BF16))

    def a_context(u):
        if u == 0:
            st["latg"] = [jnp.concatenate([t[g * _HG:(g + 1) * _HG] for t in st["lat"]], axis=0)
                          for g in range(2)]
            st["ctx"] = [jnp.zeros((_B * _HG, _D), _F32)] * 2
        for c in (2 * u, 2 * u + 1):
            st["ctx"] = [st["ctx"][g] + _dot(spread(st["latg"][g][:, c * 128:(c + 1) * 128]),
                                             slab(awuv_buf, c, g)) for g in range(2)]

    def a_out(g):
        shape = (_HG * 8, _B * _HG)
        r, c = _iota(shape, 0), _iota(shape, 1)
        perm = (((r & 7) * _HG + (r >> 3)) == c).astype(_BF16)
        t = _dot(perm, st["ctx"][g].astype(_BF16))
        lhs = jnp.concatenate([t[h * 8:(h + 1) * 8] for h in range(_HG)], axis=1)
        w = awo_buf[g * _HG:(g + 1) * _HG].reshape(_HG * _D, _M)
        o = _dot(lhs.astype(_BF16), w)
        if g == 0:
            part_ref[...] = o
        else:
            out_ref[:, 0:_M] = (part_ref[...] + o)[0:_B].astype(out_ref.dtype)

    def b_attend(pair, slot):
        b, h = pair // _H, pair % _H
        s = _dot_nt(qb_ref[h].astype(_BF16), kv_buf[slot, 0]) * scale
        p, l = softmax_parts(s)
        o = _dot(p, kv_buf[slot, 1]) / l
        ob_ref[h] = jnp.where(_iota(o.shape, 0) == b, o, ob_ref[h])

    def b_out(h0, nh):
        lhs = jnp.concatenate([ob_ref[h] for h in range(h0, h0 + nh)], axis=1)
        o = _dot(lhs.astype(_BF16), bwo_buf[h0 * _D:(h0 + nh) * _D, :])
        if h0 > 0:
            o = part_ref[...] + o
        if h0 + nh < _H:
            part_ref[...] = o
        else:
            out_ref[:, _M:2 * _M] = o[0:_B].astype(out_ref.dtype)

    head = []
    def add(make, compute):
        head.append((make(wsem.at[len(head)]), compute))

    for u in range(2):
        add(lambda s: bwq_unit(u, s), b_query if u == 1 else None)
    for u in range(2):
        add(lambda s: up_unit(awq_hbm, awq_buf, u, s), lambda u=u: a_query(u))
    for u in range(2):
        add(lambda s: up_unit(awuk_hbm, awuk_buf, u, s), lambda u=u: a_absorb(u))
    for b in range(_B):
        for u in range(2):
            add(lambda s: ckv_unit(b, u, s), lambda b=b, u=u: a_scores(b, u))
    for u in range(2):
        add(lambda s: up_unit(awuv_hbm, awuv_buf, u, s), lambda u=u: a_context(u))
    for u in range(2):
        add(lambda s: awo_unit(u, s), lambda u=u: a_out(u))
    n_head, n_pair = len(head), _B * _H
    tail = [bwo_unit(h0, nh, wsem.at[n_head + u]) for u, (h0, nh) in enumerate(_TAIL)]
    x_copies = [pltpu.make_async_copy(bx_hbm, bx_ref, xsem.at[0]),
                pltpu.make_async_copy(ax_hbm, ax_ref, xsem.at[1])]

    for cp in x_copies:
        cp.start()
    for i in range(_AHEAD):
        head[i][0].start()
    setup()
    for cp in x_copies:
        cp.wait()
    for i, (unit, compute) in enumerate(head):
        unit.wait()
        if compute is not None:
            compute()
        if i + _AHEAD < n_head:
            head[i + _AHEAD][0].start()
        else:
            kv_unit(i + _AHEAD - n_head, i + _AHEAD - n_head).start()

    def pair_step(pair, carry):
        slot = pair % _AHEAD
        kv_unit(pair, slot).wait()
        b_attend(pair, slot)

        @pl.when(pair + _AHEAD < n_pair)
        def _():
            kv_unit(pair + _AHEAD, slot).start()

        @pl.when(pair + _AHEAD == n_pair)
        def _():
            tail[0].start()

        @pl.when(pair + _AHEAD == n_pair + 1)
        def _():
            for unit in tail[1:]:
                unit.start()
        return carry

    lax.fori_loop(0, n_pair, pair_step, 0)

    for unit, (h0, nh) in zip(tail, _TAIL):
        unit.wait()
        b_out(h0, nh)


@jax.jit
def pallas_concat_heads__compressed_kv_cla__mha_block_cached__decode_kernel(
    A_x: jax.Array,
    A_c_kv: jax.Array,
    A_w_q: jax.Array,
    A_w_uk: jax.Array,
    A_w_uv: jax.Array,
    A_w_o: jax.Array,
    B_x: jax.Array,
    B_k_cache: jax.Array,
    B_v_cache: jax.Array,
    B_wq: jax.Array,
    B_wo: jax.Array,
):
    assert A_x.shape == (_B, 1, _M) and A_c_kv.shape == (_B, _SK, _DC)
    assert A_w_q.shape == (_M, _H, _D) and B_k_cache.shape == (_B, _H, _SK, _D)

    hbm = pl.BlockSpec(memory_space=pl.ANY)
    out = pl.pallas_call(
        _kernel,
        in_specs=[hbm] * 11,
        out_specs=pl.BlockSpec(memory_space=pltpu.VMEM),
        out_shape=jax.ShapeDtypeStruct((_B, 2 * _M), A_x.dtype),
        scratch_shapes=[
            pltpu.VMEM((_B, _M), _BF16),
            pltpu.VMEM((_B, _M), _BF16),
            pltpu.VMEM(A_c_kv.shape, _BF16),
            pltpu.VMEM(A_w_q.shape, _BF16),
            pltpu.VMEM(A_w_uk.shape, _BF16),
            pltpu.VMEM(A_w_uv.shape, _BF16),
            pltpu.VMEM(A_w_o.shape, _BF16),
            pltpu.VMEM(B_wq.shape, _BF16),
            pltpu.VMEM(B_wo.shape, _BF16),
            pltpu.VMEM((_AHEAD, 2, _SK, _D), _BF16),
            pltpu.VMEM((128, 128 * _HG), _BF16),
            pltpu.VMEM((_H, 8, _D), _F32),
            pltpu.VMEM((_H, 8, _D), _F32),
            pltpu.VMEM((8, _M), _F32),
            pltpu.SemaphoreType.DMA((2,)),
            pltpu.SemaphoreType.DMA((18 + len(_TAIL),)),
            pltpu.SemaphoreType.DMA((_AHEAD,)),
        ],
        compiler_params=pltpu.CompilerParams(vmem_limit_bytes=96 * 1024 * 1024),
    )(A_x.reshape(_B, _M), A_c_kv, A_w_q, A_w_uk, A_w_uv, A_w_o,
      B_x.reshape(_B, _M), B_k_cache, B_v_cache, B_wq, B_wo)
    return out.reshape(_B, 1, 2 * _M)
```

```python
import jax
import jax.numpy as jnp
from jax import lax
import jax.experimental.pallas as pl
import jax.experimental.pallas.tpu as pltpu

_B, _H, _SK, _D, _M, _DC = 4, 32, 4096, 128, 512, 512
_HG = 16
_NS = 4
_NPOS = 128
_STEP = 32
_SPG = _NPOS // _STEP
_LAG = _SPG + 1
_SLOTS = 3
_HS = _H // _NS
_F32, _BF16 = jnp.float32, jnp.bfloat16
_NT = (((1,), (1,)), ((), ()))


def _dot(a, b):
    return jnp.dot(a, b, preferred_element_type=_F32)


def _dot_nt(a, b):
    return lax.dot_general(a, b, _NT, preferred_element_type=_F32)


def _iota(shape, dim):
    return lax.broadcasted_iota(jnp.int32, shape, dim)


def _ds(start, size):
    return pl.ds(pl.multiple_of(start, size), size)


def _kernel(ax_hbm, ckv_hbm, awq_hbm, awuk_hbm, awuv_hbm, awo_hbm,
            bx_hbm, k_hbm, v_hbm, bwq_hbm, bwo_hbm,
            out_ref,
            ax_ref, bx_ref, ckv_buf, awq_buf, awuk_buf, awuv_buf, awo_buf, bwq_buf, bwo_buf,
            kv_buf, e_ref, qb_ref, oa_ref, ob_ref, part_ref, xsem, wsem, kvsem, tsem):
    scale = _D ** -0.5

    def up_window(j):
        return (slice(None), pl.ds(j, 1))

    def wide_window(j):
        return (slice(None), _ds((j // 8) * 8, 8), _ds((j % 8) * 512, 512))

    def tall_window(j):
        return (slice(None), _ds(j * 8, 8))

    def kv_window(j):
        return (slice(None), _ds(j * 32, 32))

    def issue(blocks, first, count):
        def body(j, carry):
            for queue, (src, dst, window, sem) in enumerate(blocks):
                w = window(first + j)
                pltpu.make_async_copy(src.at[w], dst.at[w], sem).start(priority=queue)
            return carry
        lax.fori_loop(0, count, body, 0)

    def wait_filled(dst, sem):
        pltpu.make_async_copy(dst, dst, sem).wait()

    head_groups = [
        [(awq_hbm, awq_buf, up_window), (awuk_hbm, awuk_buf, up_window)],
        [(ckv_hbm.at[0], ckv_buf.at[0], tall_window), (ckv_hbm.at[1], ckv_buf.at[1], tall_window)],
        [(ckv_hbm.at[2], ckv_buf.at[2], tall_window), (ckv_hbm.at[3], ckv_buf.at[3], tall_window)],
        [(awuv_hbm, awuv_buf, up_window), (bwq_hbm, bwq_buf, wide_window)],
    ]
    head_groups = [[blk + (wsem.at[2 * g + q],) for q, blk in enumerate(grp)]
                   for g, grp in enumerate(head_groups)]

    def issue_kv(step):
        g = step // _SPG
        slot = g % _SLOTS
        issue([(hbm.at[g], kv_buf.at[slot, q], kv_window, kvsem.at[2 * slot + q])
               for q, hbm in enumerate((k_hbm, v_hbm))], (step % _SPG) * _STEP, _STEP)

    def issue_tail(step):
        per = _NPOS // _HS
        for i in range(step * _STEP // per, (step + 1) * _STEP // per):
            issue([(awo_hbm, awo_buf, tall_window, tsem.at[2 * i]),
                   (bwo_hbm, bwo_buf, tall_window, tsem.at[2 * i + 1])], i * per, per)

    def head_diag(t):
        keep = (_iota(t.shape, 0) & (_HG - 1)) == (_iota(t.shape, 1) & (_HG - 1))
        return jnp.where(keep, t, 0.0).astype(_BF16)

    def spread(x):
        return head_diag(_dot(x, e_ref[...]))

    def slab(buf, c, g):
        return buf[c, :, g * _HG:(g + 1) * _HG, :].reshape(128 * _HG, _D)

    st = {}

    def setup():
        e_ref[...] = ((_iota(e_ref.shape, 1) // _HG) == _iota(e_ref.shape, 0)).astype(_BF16)
        ob_ref[...] = jnp.zeros(ob_ref.shape, _F32)

    def a_query(u):
        if u == 0:
            ax = ax_ref[...].astype(_F32)
            st["x"] = jnp.concatenate(
                [jnp.broadcast_to(ax[b:b + 1], (_HG, _M)) for b in range(_B)],
                axis=0).astype(_BF16)
            st["q"] = [jnp.zeros((_B * _HG, _D), _F32)] * 2
        for c in (2 * u, 2 * u + 1):
            lhs = spread(st["x"][:, c * 128:(c + 1) * 128])
            st["q"] = [st["q"][g] + _dot(lhs, slab(awq_buf, c, g)) for g in range(2)]

    def a_absorb(u):
        if u == 0:
            st["qabs"] = [[], []]
        for c in (2 * u, 2 * u + 1):
            for g in range(2):
                t = head_diag(_dot_nt(st["q"][g].astype(_BF16), slab(awuk_buf, c, g)))
                st["qabs"][g].append(_dot_nt(t, e_ref[...]).astype(_BF16))

    def a_attend(b, u):
        if u == 0:
            st["qb"] = jnp.concatenate(
                [jnp.concatenate([t[b * _HG:(b + 1) * _HG] for t in st["qabs"][g]], axis=1)
                 for g in range(2)], axis=0)
        c = ckv_buf[b, 2 * u:2 * u + 2].reshape(_SK // 2, _DC)
        s = _dot_nt(st["qb"], c) * scale
        m = jnp.max(s, axis=-1, keepdims=True)
        if u == 0:
            p = jnp.exp(s - m)
            st["m"], st["l"] = m, jnp.sum(p, axis=-1, keepdims=True)
            st["acc"] = _dot(p.astype(_BF16), c)
        else:
            m = jnp.maximum(m, st["m"])
            alpha = jnp.exp(st["m"] - m)
            p = jnp.exp(s - m)
            l = alpha * st["l"] + jnp.sum(p, axis=-1, keepdims=True)
            acc = alpha * st["acc"] + _dot(p.astype(_BF16), c)
            st.setdefault("lat", []).append((acc / l).astype(_BF16))

    def a_context(u):
        if u == 0:
            st["latg"] = [jnp.concatenate([t[g * _HG:(g + 1) * _HG] for t in st["lat"]], axis=0)
                          for g in range(2)]
            st["ctx"] = [jnp.zeros((_B * _HG, _D), _F32)] * 2
        for c in (2 * u, 2 * u + 1):
            st["ctx"] = [st["ctx"][g] + _dot(spread(st["latg"][g][:, c * 128:(c + 1) * 128]),
                                             slab(awuv_buf, c, g)) for g in range(2)]

    def a_regroup():
        shape = (_HG * 8, _B * _HG)
        r, c = _iota(shape, 0), _iota(shape, 1)
        perm = (((r & 7) * _HG + (r >> 3)) == c).astype(_BF16)
        for g in range(2):
            t = _dot(perm, st["ctx"][g].astype(_BF16))
            oa_ref[g * _HG:(g + 1) * _HG] = t.reshape(_HG, 8, _D)

    def b_query():
        row = _iota((8, _M), 0)
        bx = bx_ref[...].astype(_F32)
        x = jnp.zeros((8, _M), _F32)
        for b in range(_B):
            x = jnp.where(row == b, bx[b:b + 1], x)
        q = _dot(x.astype(_BF16), bwq_buf[...].reshape(_M, _H * _D))
        for h in range(_H):
            qb_ref[h] = q[:, h * _D:(h + 1) * _D]

    def b_attend(pair, slot):
        b, h, i = pair // _H, pair % _H, pair % _NS
        s = _dot_nt(qb_ref[h].astype(_BF16), kv_buf[slot, 0, i]) * scale
        p = jnp.exp(s - jnp.max(s, axis=-1, keepdims=True))
        l = jnp.sum(p, axis=-1, keepdims=True)
        o = _dot(p.astype(_BF16), kv_buf[slot, 1, i]) / l
        ob_ref[h] = jnp.where(_iota(o.shape, 0) == b, o, ob_ref[h])

    def project(i):
        sl = slice(i * _D, (i + 1) * _D)
        outs = []
        for q, (o_ref, w_buf) in enumerate(((oa_ref, awo_buf), (ob_ref, bwo_buf))):
            wait_filled(w_buf.at[:, sl], tsem.at[2 * i + q])
            lhs = jnp.concatenate([o_ref[s * _HS + i] for s in range(_NS)], axis=1)
            outs.append(_dot(lhs.astype(_BF16), w_buf[:, sl, :].reshape(_NS * _D, _M)))
        o = jnp.concatenate(outs, axis=1)
        if i > 0:
            o = part_ref[...] + o
        if i < _HS - 1:
            part_ref[...] = o
        else:
            out_ref[...] = o[0:_B].astype(out_ref.dtype)

    pieces = [lambda: a_query(0), lambda: a_query(1), lambda: a_absorb(0), lambda: a_absorb(1)]
    pieces += [lambda b=b, u=u: a_attend(b, u) for b in range(_B) for u in range(2)]
    pieces += [lambda: a_context(0), lambda: a_context(1), a_regroup, b_query]
    n_head, n_pair = len(head_groups) * _SPG, _B * _H
    assert len(pieces) == n_head and _NS == _SPG

    x_copies = [pltpu.make_async_copy(ax_hbm, ax_ref, xsem.at[0]),
                pltpu.make_async_copy(bx_hbm, bx_ref, xsem.at[1])]
    for cp in x_copies:
        cp.start()
    for step in range(n_head + _LAG + 1):
        if step < n_head:
            issue(head_groups[step // _SPG], (step % _SPG) * _STEP, _STEP)
        else:
            issue_kv(step - n_head)
        if step == 1:
            setup()
            for cp in x_copies:
                cp.wait()
        i = step - _LAG
        if 0 <= i < n_head:
            if i % _SPG == 0:
                for _, dst, _, sem in head_groups[i // _SPG]:
                    wait_filled(dst, sem)
            pieces[i]()

    def pair_step(pair, carry):
        slot = (pair // _NS) % _SLOTS

        @pl.when(pair % _NS == 0)
        def _():
            for q in range(2):
                wait_filled(kv_buf.at[slot, q], kvsem.at[2 * slot + q])

        b_attend(pair, slot)
        nxt = pair + _LAG + 1

        @pl.when(nxt < n_pair)
        def _():
            issue_kv(nxt)

        for t in range(_SPG):
            @pl.when(nxt == n_pair + t)
            def _():
                issue_tail(t)
        return carry

    lax.fori_loop(0, n_pair, pair_step, 0)

    for i in range(_HS):
        project(i)


@jax.jit
def pallas_concat_heads__compressed_kv_cla__mha_block_cached__decode_kernel(
    A_x: jax.Array,
    A_c_kv: jax.Array,
    A_w_q: jax.Array,
    A_w_uk: jax.Array,
    A_w_uv: jax.Array,
    A_w_o: jax.Array,
    B_x: jax.Array,
    B_k_cache: jax.Array,
    B_v_cache: jax.Array,
    B_wq: jax.Array,
    B_wo: jax.Array,
):
    assert A_x.shape == (_B, 1, _M) and A_c_kv.shape == (_B, _SK, _DC)
    assert A_w_q.shape == (_M, _H, _D) and B_k_cache.shape == (_B, _H, _SK, _D)

    up = (_NS, _M // _NS, _H, _D)
    tall = (_NS, _H * _D // _NS, _M)
    wide = (_NS, _M // _NS, _H * _D)
    ckv = (_B, _NS, _SK // _NS, _DC)
    kv = (_B * _H // _NS, _NS, _SK, _D)

    out = pl.pallas_call(
        _kernel,
        in_specs=[pl.BlockSpec(memory_space=pl.ANY)] * 11,
        out_specs=pl.BlockSpec(memory_space=pltpu.VMEM),
        out_shape=jax.ShapeDtypeStruct((_B, 2 * _M), A_x.dtype),
        scratch_shapes=[
            pltpu.VMEM((_B, _M), _BF16),
            pltpu.VMEM((_B, _M), _BF16),
            pltpu.VMEM(ckv, _BF16),
            pltpu.VMEM(up, _BF16),
            pltpu.VMEM(up, _BF16),
            pltpu.VMEM(up, _BF16),
            pltpu.VMEM(tall, _BF16),
            pltpu.VMEM(wide, _BF16),
            pltpu.VMEM(tall, _BF16),
            pltpu.VMEM((_SLOTS, 2) + kv[1:], _BF16),
            pltpu.VMEM((128, 128 * _HG), _BF16),
            pltpu.VMEM((_H, 8, _D), _F32),
            pltpu.VMEM((_H, 8, _D), _F32),
            pltpu.VMEM((_H, 8, _D), _F32),
            pltpu.VMEM((8, 2 * _M), _F32),
            pltpu.SemaphoreType.DMA((2,)),
            pltpu.SemaphoreType.DMA((8,)),
            pltpu.SemaphoreType.DMA((2 * _SLOTS,)),
            pltpu.SemaphoreType.DMA((2 * _HS,)),
        ],
        compiler_params=pltpu.CompilerParams(vmem_limit_bytes=100 * 1024 * 1024),
    )(A_x.reshape(_B, _M), A_c_kv.reshape(ckv), A_w_q.reshape(up), A_w_uk.reshape(up),
      A_w_uv.reshape(up), A_w_o.reshape(tall), B_x.reshape(_B, _M), B_k_cache.reshape(kv),
      B_v_cache.reshape(kv), B_wq.reshape(wide), B_wo.reshape(tall))
    return out.reshape(_B, 1, 2 * _M)
```

```python
import jax
import jax.numpy as jnp
from jax import lax
import jax.experimental.pallas as pl
import jax.experimental.pallas.tpu as pltpu

_B, _H, _SK, _D, _M, _DC = 4, 32, 4096, 128, 512, 512
_HG = 16
_NS = 4
_NPOS = 128
_STEP = 32
_SPG = _NPOS // _STEP
_LAG = _SPG + 1
_SLOTS = 3
_HS = _H // _NS
_F32, _BF16 = jnp.float32, jnp.bfloat16
_NT = (((1,), (1,)), ((), ()))


def _dot(a, b):
    return jnp.dot(a, b, preferred_element_type=_F32)


def _dot_nt(a, b):
    return lax.dot_general(a, b, _NT, preferred_element_type=_F32)


def _iota(shape, dim):
    return lax.broadcasted_iota(jnp.int32, shape, dim)


def _ds(start, size):
    return pl.ds(pl.multiple_of(start, size), size)


def _kernel(ax_hbm, ckv_hbm, awq_hbm, awuk_hbm, awuv_hbm, awo_hbm,
            bx_hbm, k_hbm, v_hbm, bwq_hbm, bwo_hbm,
            out_ref,
            ax_ref, bx_ref, ckv_buf, awq_buf, awuk_buf, awuv_buf, awo_buf, bwq_buf, bwo_buf,
            kv_buf, e_ref, qb_ref, oa_ref, ob_ref, part_ref, xsem, wsem, kvsem, tsem):
    scale = _D ** -0.5

    def up_window(j):
        return (slice(None), pl.ds(j, 1))

    def wide_window(j):
        return (slice(None), _ds((j // 8) * 8, 8), _ds((j % 8) * 512, 512))

    def tall_window(j):
        return (slice(None), _ds(j * 8, 8))

    def kv_window(j):
        return (slice(None), _ds(j * 32, 32))

    def issue(blocks, first, count):
        def body(i, carry):
            j = first + i
            for queue, (src, dst, window, sem) in enumerate(blocks):
                w = window((j % 2) * (_NPOS // 2) + j // 2)
                pltpu.make_async_copy(src.at[w], dst.at[w], sem).start(priority=queue)
            return carry
        lax.fori_loop(0, count, body, 0)

    def wait_filled(dst, sem):
        pltpu.make_async_copy(dst, dst, sem).wait()

    head_groups = [
        [(awq_hbm, awq_buf, up_window), (awuk_hbm, awuk_buf, up_window)],
        [(ckv_hbm.at[0], ckv_buf.at[0], tall_window), (ckv_hbm.at[1], ckv_buf.at[1], tall_window)],
        [(ckv_hbm.at[2], ckv_buf.at[2], tall_window), (ckv_hbm.at[3], ckv_buf.at[3], tall_window)],
        [(awuv_hbm, awuv_buf, up_window), (bwq_hbm, bwq_buf, wide_window)],
    ]
    head_groups = [[blk + (wsem.at[2 * g + q],) for q, blk in enumerate(grp)]
                   for g, grp in enumerate(head_groups)]

    def issue_kv(step):
        g = step // _SPG
        slot = g % _SLOTS
        issue([(hbm.at[g], kv_buf.at[slot, q], kv_window, kvsem.at[2 * slot + q])
               for q, hbm in enumerate((k_hbm, v_hbm))], (step % _SPG) * _STEP, _STEP)

    def issue_tail(step):
        issue([(awo_hbm, awo_buf, tall_window, tsem.at[2 * step]),
               (bwo_hbm, bwo_buf, tall_window, tsem.at[2 * step + 1])], step * _STEP, _STEP)

    def head_diag(t):
        keep = (_iota(t.shape, 0) & (_HG - 1)) == (_iota(t.shape, 1) & (_HG - 1))
        return jnp.where(keep, t, 0.0).astype(_BF16)

    def spread(x):
        return head_diag(_dot(x, e_ref[...]))

    def slab(buf, c, g):
        return buf[c, :, g * _HG:(g + 1) * _HG, :].reshape(128 * _HG, _D)

    st = {}

    def setup():
        e_ref[...] = ((_iota(e_ref.shape, 1) // _HG) == _iota(e_ref.shape, 0)).astype(_BF16)
        ob_ref[...] = jnp.zeros(ob_ref.shape, _F32)

    def a_query(u):
        if u == 0:
            ax = ax_ref[...].astype(_F32)
            st["x"] = jnp.concatenate(
                [jnp.broadcast_to(ax[b:b + 1], (_HG, _M)) for b in range(_B)],
                axis=0).astype(_BF16)
            st["q"] = [jnp.zeros((_B * _HG, _D), _F32)] * 2
        for c in (2 * u, 2 * u + 1):
            lhs = spread(st["x"][:, c * 128:(c + 1) * 128])
            st["q"] = [st["q"][g] + _dot(lhs, slab(awq_buf, c, g)) for g in range(2)]

    def a_absorb(u):
        if u == 0:
            st["qabs"] = [[], []]
        for c in (2 * u, 2 * u + 1):
            for g in range(2):
                t = head_diag(_dot_nt(st["q"][g].astype(_BF16), slab(awuk_buf, c, g)))
                st["qabs"][g].append(_dot_nt(t, e_ref[...]).astype(_BF16))

    def a_attend(b, u):
        if u == 0:
            st["qb"] = jnp.concatenate(
                [jnp.concatenate([t[b * _HG:(b + 1) * _HG] for t in st["qabs"][g]], axis=1)
                 for g in range(2)], axis=0)
        c = ckv_buf[b, 2 * u:2 * u + 2].reshape(_SK // 2, _DC)
        s = _dot_nt(st["qb"], c) * scale
        m = jnp.max(s, axis=-1, keepdims=True)
        if u == 0:
            p = jnp.exp(s - m)
            st["m"], st["l"] = m, jnp.sum(p, axis=-1, keepdims=True)
            st["acc"] = _dot(p.astype(_BF16), c)
        else:
            m = jnp.maximum(m, st["m"])
            alpha = jnp.exp(st["m"] - m)
            p = jnp.exp(s - m)
            l = alpha * st["l"] + jnp.sum(p, axis=-1, keepdims=True)
            acc = alpha * st["acc"] + _dot(p.astype(_BF16), c)
            st.setdefault("lat", []).append((acc / l).astype(_BF16))

    def a_context(u):
        if u == 0:
            st["latg"] = [jnp.concatenate([t[g * _HG:(g + 1) * _HG] for t in st["lat"]], axis=0)
                          for g in range(2)]
            st["ctx"] = [jnp.zeros((_B * _HG, _D), _F32)] * 2
        for c in (2 * u, 2 * u + 1):
            st["ctx"] = [st["ctx"][g] + _dot(spread(st["latg"][g][:, c * 128:(c + 1) * 128]),
                                             slab(awuv_buf, c, g)) for g in range(2)]

    def a_regroup():
        shape = (_HG * 8, _B * _HG)
        r, c = _iota(shape, 0), _iota(shape, 1)
        perm = (((r & 7) * _HG + (r >> 3)) == c).astype(_BF16)
        for g in range(2):
            t = _dot(perm, st["ctx"][g].astype(_BF16))
            oa_ref[g * _HG:(g + 1) * _HG] = t.reshape(_HG, 8, _D)

    def b_query():
        row = _iota((8, _M), 0)
        bx = bx_ref[...].astype(_F32)
        x = jnp.zeros((8, _M), _F32)
        for b in range(_B):
            x = jnp.where(row == b, bx[b:b + 1], x)
        q = _dot(x.astype(_BF16), bwq_buf[...].reshape(_M, _H * _D))
        for h in range(_H):
            qb_ref[h] = q[:, h * _D:(h + 1) * _D]

    def b_attend(pair, slot):
        b, h, i = pair // _H, pair % _H, pair % _NS
        s = _dot_nt(qb_ref[h].astype(_BF16), kv_buf[slot, 0, i]) * scale
        p = jnp.exp(s - jnp.max(s, axis=-1, keepdims=True))
        l = jnp.sum(p, axis=-1, keepdims=True)
        o = _dot(p.astype(_BF16), kv_buf[slot, 1, i]) / l
        ob_ref[h] = jnp.where(_iota(o.shape, 0) == b, o, ob_ref[h])

    def project(step):
        heads = (step, step + _HS // 2)
        outs = []
        for q, (o_ref, w_buf) in enumerate(((oa_ref, awo_buf), (ob_ref, bwo_buf))):
            for i in heads:
                wait_filled(w_buf.at[:, i * _D:(i + 1) * _D], tsem.at[2 * step + q])
            o = 0.0
            for i in heads:
                lhs = jnp.concatenate([o_ref[s * _HS + i] for s in range(_NS)], axis=1)
                w = w_buf[:, i * _D:(i + 1) * _D, :].reshape(_NS * _D, _M)
                o = o + _dot(lhs.astype(_BF16), w)
            outs.append(o)
        o = jnp.concatenate(outs, axis=1)
        if step > 0:
            o = part_ref[...] + o
        if step < _SPG - 1:
            part_ref[...] = o
        else:
            out_ref[...] = o[0:_B].astype(out_ref.dtype)

    pieces = [lambda: a_query(0), lambda: a_query(1), lambda: a_absorb(0), lambda: a_absorb(1)]
    pieces += [lambda b=b, u=u: a_attend(b, u) for b in range(_B) for u in range(2)]
    pieces += [lambda: a_context(0), lambda: a_context(1), a_regroup, b_query]
    n_head, n_pair = len(head_groups) * _SPG, _B * _H
    assert len(pieces) == n_head and _NS == _SPG

    x_copies = [pltpu.make_async_copy(ax_hbm, ax_ref, xsem.at[0]),
                pltpu.make_async_copy(bx_hbm, bx_ref, xsem.at[1])]
    for cp in x_copies:
        cp.start()
    for step in range(n_head + _LAG + 1):
        if step < n_head:
            issue(head_groups[step // _SPG], (step % _SPG) * _STEP, _STEP)
        else:
            issue_kv(step - n_head)
        if step == 1:
            setup()
            for cp in x_copies:
                cp.wait()
        i = step - _LAG
        if 0 <= i < n_head:
            if i % _SPG == 0:
                for _, dst, _, sem in head_groups[i // _SPG]:
                    wait_filled(dst, sem)
            pieces[i]()

    def pair_step(pair, carry):
        slot = (pair // _NS) % _SLOTS

        @pl.when(pair % _NS == 0)
        def _():
            for q in range(2):
                wait_filled(kv_buf.at[slot, q], kvsem.at[2 * slot + q])

        b_attend(pair, slot)
        nxt = pair + _LAG + 1

        @pl.when(nxt < n_pair)
        def _():
            issue_kv(nxt)

        for t in range(_SPG):
            @pl.when(nxt == n_pair + t)
            def _():
                issue_tail(t)
        return carry

    lax.fori_loop(0, n_pair, pair_step, 0)

    for t in range(_SPG):
        project(t)


@jax.jit
def pallas_concat_heads__compressed_kv_cla__mha_block_cached__decode_kernel(
    A_x: jax.Array,
    A_c_kv: jax.Array,
    A_w_q: jax.Array,
    A_w_uk: jax.Array,
    A_w_uv: jax.Array,
    A_w_o: jax.Array,
    B_x: jax.Array,
    B_k_cache: jax.Array,
    B_v_cache: jax.Array,
    B_wq: jax.Array,
    B_wo: jax.Array,
):
    assert A_x.shape == (_B, 1, _M) and A_c_kv.shape == (_B, _SK, _DC)
    assert A_w_q.shape == (_M, _H, _D) and B_k_cache.shape == (_B, _H, _SK, _D)

    up = (_NS, _M // _NS, _H, _D)
    tall = (_NS, _H * _D // _NS, _M)
    wide = (_NS, _M // _NS, _H * _D)
    ckv = (_B, _NS, _SK // _NS, _DC)
    kv = (_B * _H // _NS, _NS, _SK, _D)

    out = pl.pallas_call(
        _kernel,
        in_specs=[pl.BlockSpec(memory_space=pl.ANY)] * 11,
        out_specs=pl.BlockSpec(memory_space=pltpu.VMEM),
        out_shape=jax.ShapeDtypeStruct((_B, 2 * _M), A_x.dtype),
        scratch_shapes=[
            pltpu.VMEM((_B, _M), _BF16),
            pltpu.VMEM((_B, _M), _BF16),
            pltpu.VMEM(ckv, _BF16),
            pltpu.VMEM(up, _BF16),
            pltpu.VMEM(up, _BF16),
            pltpu.VMEM(up, _BF16),
            pltpu.VMEM(tall, _BF16),
            pltpu.VMEM(wide, _BF16),
            pltpu.VMEM(tall, _BF16),
            pltpu.VMEM((_SLOTS, 2) + kv[1:], _BF16),
            pltpu.VMEM((128, 128 * _HG), _BF16),
            pltpu.VMEM((_H, 8, _D), _F32),
            pltpu.VMEM((_H, 8, _D), _F32),
            pltpu.VMEM((_H, 8, _D), _F32),
            pltpu.VMEM((8, 2 * _M), _F32),
            pltpu.SemaphoreType.DMA((2,)),
            pltpu.SemaphoreType.DMA((8,)),
            pltpu.SemaphoreType.DMA((2 * _SLOTS,)),
            pltpu.SemaphoreType.DMA((2 * _SPG,)),
        ],
        compiler_params=pltpu.CompilerParams(vmem_limit_bytes=100 * 1024 * 1024),
    )(A_x.reshape(_B, _M), A_c_kv.reshape(ckv), A_w_q.reshape(up), A_w_uk.reshape(up),
      A_w_uv.reshape(up), A_w_o.reshape(tall), B_x.reshape(_B, _M), B_k_cache.reshape(kv),
      B_v_cache.reshape(kv), B_wq.reshape(wide), B_wo.reshape(tall))
    return out.reshape(_B, 1, 2 * _M)
```

```python
import jax
import jax.numpy as jnp
from jax import lax
import jax.experimental.pallas as pl
import jax.experimental.pallas.tpu as pltpu

_B, _H, _SK, _D, _M, _DC = 4, 32, 4096, 128, 512, 512
_HG = 16
_SLAB = 1 << 19
_NPOS = 64
_G = 8
_SLOTS = 3
_WS = 4
_HS = _H // _WS
_F32, _BF16 = jnp.float32, jnp.bfloat16
_NT = (((1,), (1,)), ((), ()))


def _dot(a, b):
    return jnp.dot(a, b, preferred_element_type=_F32)


def _dot_nt(a, b):
    return lax.dot_general(a, b, _NT, preferred_element_type=_F32)


def _iota(shape, dim):
    return lax.broadcasted_iota(jnp.int32, shape, dim)


def _ds(start, size):
    return pl.ds(pl.multiple_of(start, size), size)


def _kernel(ax_hbm, ckv_hbm, awq_hbm, awuk_hbm, awuv_hbm, awo_hbm,
            bx_hbm, k_hbm, v_hbm, bwq_hbm, bwo_hbm,
            out_ref,
            ax_ref, bx_ref, ckv_buf, awq_buf, awuk_buf, awuv_buf, awo_buf, bwq_buf, bwo_buf,
            kv_buf, e_ref, qb_ref, oa_ref, ob_ref, part_ref, xsem, wsem, kvsem, hsem, tsem):
    scale = _D ** -0.5

    def up_window(j):
        return (_ds(j * 2, 2),)

    def wide_window(j):
        return (_ds((j // 4) * 8, 8), _ds((j % 4) * 1024, 1024))

    def tall_window(j):
        return (_ds(j * 16, 16),)

    def kv_window(j):
        return (_ds(j * 64, 64),)

    def issue(blocks, first, count):
        def body(j, carry):
            for t in range(0, blocks[0][0].shape[0], 2):
                for queue, (src, dst, window, sem) in enumerate(blocks):
                    w = (pl.ds(t, 2),) + window(first + j)
                    pltpu.make_async_copy(src.at[w], dst.at[w], sem).start(priority=queue)
            return carry
        lax.fori_loop(0, count, body, 0)

    def wait_filled(dst, sem):
        pltpu.make_async_copy(dst, dst, sem).wait()

    head_groups = [
        [(awq_hbm, awq_buf, up_window), (awuk_hbm, awuk_buf, up_window)],
        [(ckv_hbm.at[q], ckv_buf.at[q], tall_window) for q in range(2)],
        [(awuv_hbm, awuv_buf, up_window), (bwq_hbm, bwq_buf, wide_window)],
    ]
    head_groups = [[blk + (wsem.at[2 * g + q],) for q, blk in enumerate(grp)]
                   for g, grp in enumerate(head_groups)]

    def kv_group(g):
        slot = g % _SLOTS
        return [(hbm.at[g], kv_buf.at[slot, q], kv_window, kvsem.at[2 * slot + q])
                for q, hbm in enumerate((k_hbm, v_hbm))]

    def kv_half(g, i):
        sl = pl.ds(i * (_G // 2), _G // 2)
        return [(src.at[sl], dst.at[sl], window, hsem.at[2 * i + q])
                for q, (src, dst, window, _) in enumerate(kv_group(g))]

    def issue_step(group, t):
        per = _NPOS // group[0][0].shape[0]
        issue(group, t * per, per)

    def wait_group(group):
        for _, dst, _, sem in group:
            wait_filled(dst, sem)

    def issue_tail(step):
        per, n = _NPOS // _HS, _HS // _WS
        for i in range(step * n, (step + 1) * n):
            issue([(awo_hbm, awo_buf, tall_window, tsem.at[2 * i]),
                   (bwo_hbm, bwo_buf, tall_window, tsem.at[2 * i + 1])], i * per, per)

    def head_diag(t):
        keep = (_iota(t.shape, 0) & (_HG - 1)) == (_iota(t.shape, 1) & (_HG - 1))
        return jnp.where(keep, t, 0.0).astype(_BF16)

    def spread(x):
        return head_diag(_dot(x, e_ref[...]))

    def slab(buf, c, g):
        return buf[c, :, g * _HG:(g + 1) * _HG, :].reshape(128 * _HG, _D)

    st = {}

    def setup():
        e_ref[...] = ((_iota(e_ref.shape, 1) // _HG) == _iota(e_ref.shape, 0)).astype(_BF16)
        ob_ref[...] = jnp.zeros(ob_ref.shape, _F32)

    def a_query(u):
        if u == 0:
            ax = ax_ref[...].astype(_F32)
            st["x"] = jnp.concatenate(
                [jnp.broadcast_to(ax[b:b + 1], (_HG, _M)) for b in range(_B)],
                axis=0).astype(_BF16)
            st["q"] = [jnp.zeros((_B * _HG, _D), _F32)] * 2
        for c in (2 * u, 2 * u + 1):
            lhs = spread(st["x"][:, c * 128:(c + 1) * 128])
            st["q"] = [st["q"][g] + _dot(lhs, slab(awq_buf, c, g)) for g in range(2)]

    def a_absorb(u):
        if u == 0:
            st["qabs"] = [[], []]
        for c in (2 * u, 2 * u + 1):
            for g in range(2):
                t = head_diag(_dot_nt(st["q"][g].astype(_BF16), slab(awuk_buf, c, g)))
                st["qabs"][g].append(_dot_nt(t, e_ref[...]).astype(_BF16))

    def a_attend(b, u):
        if u == 0:
            st["qb"] = jnp.concatenate(
                [jnp.concatenate([t[b * _HG:(b + 1) * _HG] for t in st["qabs"][g]], axis=1)
                 for g in range(2)], axis=0)
        first = (b % 2) * 4 + 2 * u
        c = ckv_buf[b // 2, first:first + 2].reshape(_SK // 2, _DC)
        s = _dot_nt(st["qb"], c) * scale
        m = jnp.max(s, axis=-1, keepdims=True)
        if u == 0:
            p = jnp.exp(s - m)
            st["m"], st["l"] = m, jnp.sum(p, axis=-1, keepdims=True)
            st["acc"] = _dot(p.astype(_BF16), c)
        else:
            m = jnp.maximum(m, st["m"])
            alpha = jnp.exp(st["m"] - m)
            p = jnp.exp(s - m)
            l = alpha * st["l"] + jnp.sum(p, axis=-1, keepdims=True)
            acc = alpha * st["acc"] + _dot(p.astype(_BF16), c)
            st.setdefault("lat", []).append((acc / l).astype(_BF16))

    def a_context(u):
        if u == 0:
            st["latg"] = [jnp.concatenate([t[g * _HG:(g + 1) * _HG] for t in st["lat"]], axis=0)
                          for g in range(2)]
            st["ctx"] = [jnp.zeros((_B * _HG, _D), _F32)] * 2
        for c in (2 * u, 2 * u + 1):
            st["ctx"] = [st["ctx"][g] + _dot(spread(st["latg"][g][:, c * 128:(c + 1) * 128]),
                                             slab(awuv_buf, c, g)) for g in range(2)]

    def a_regroup():
        shape = (_HG * 8, _B * _HG)
        r, c = _iota(shape, 0), _iota(shape, 1)
        perm = (((r & 7) * _HG + (r >> 3)) == c).astype(_BF16)
        for g in range(2):
            t = _dot(perm, st["ctx"][g].astype(_BF16))
            oa_ref[g * _HG:(g + 1) * _HG] = t.reshape(_HG, 8, _D)

    def b_query():
        row = _iota((8, _M), 0)
        bx = bx_ref[...].astype(_F32)
        x = jnp.zeros((8, _M), _F32)
        for b in range(_B):
            x = jnp.where(row == b, bx[b:b + 1], x)
        q = _dot(x.astype(_BF16), bwq_buf[...].reshape(_M, _H * _D))
        for h in range(_H):
            qb_ref[h] = q[:, h * _D:(h + 1) * _D]

    def b_attend(pair):
        b, h, slot, i = pair // _H, pair % _H, (pair // _G) % _SLOTS, pair % _G
        s = _dot_nt(qb_ref[h].astype(_BF16), kv_buf[slot, 0, i]) * scale
        p = jnp.exp(s - jnp.max(s, axis=-1, keepdims=True))
        l = jnp.sum(p, axis=-1, keepdims=True)
        o = _dot(p.astype(_BF16), kv_buf[slot, 1, i]) / l
        ob_ref[h] = jnp.where(_iota(o.shape, 0) == b, o, ob_ref[h])

    def project(i):
        sl = slice(i * _D, (i + 1) * _D)
        outs = []
        for q, (o_ref, w_buf) in enumerate(((oa_ref, awo_buf), (ob_ref, bwo_buf))):
            wait_filled(w_buf.at[:, sl], tsem.at[2 * i + q])
            lhs = jnp.concatenate([o_ref[s * _HS + i] for s in range(_WS)], axis=1)
            outs.append(_dot(lhs.astype(_BF16), w_buf[:, sl, :].reshape(_WS * _D, _M)))
        o = jnp.concatenate(outs, axis=1)
        if i > 0:
            o = part_ref[...] + o
        if i < _HS - 1:
            part_ref[...] = o
        else:
            out_ref[...] = o[0:_B].astype(out_ref.dtype)

    pieces = [
        [lambda: a_query(0), lambda: a_query(1), lambda: a_absorb(0), lambda: a_absorb(1)],
        [lambda b=b, u=u: a_attend(b, u) for b in range(_B) for u in range(2)],
        [lambda: a_context(0), lambda: a_context(1), a_regroup, b_query],
    ]
    steps, ready = [], {}
    for g, grp in enumerate(head_groups):
        steps += [(grp, t) for t in range(grp[0][0].shape[0])]
        ready[len(steps) + 1] = g
    steps += [(kv_group(t // _G), t % _G) for t in range(_G + 2)]

    x_copies = [pltpu.make_async_copy(ax_hbm, ax_ref, xsem.at[0]),
                pltpu.make_async_copy(bx_hbm, bx_ref, xsem.at[1])]
    for cp in x_copies:
        cp.start()
    todo = []
    for i, step in enumerate(steps):
        issue_step(*step)
        if i == 1:
            setup()
            for cp in x_copies:
                cp.wait()
        if i in ready:
            wait_group(head_groups[ready[i]])
            todo += pieces[ready[i]]
        if todo:
            todo.pop(0)()
    assert not todo

    def attend_two(pair):
        for i in range(2):
            b_attend(pair + i)

    last = _B * _H // _G - 1

    def group_step(g, carry):
        wait_group(kv_group(g))

        def busy(t, c):
            attend_two(g * _G + 2 * t)
            issue_step(kv_group(g + 1), t + 2)
            return c
        lax.fori_loop(0, _G // 2, busy, 0)
        for t in range(_G // 2 + 2, _G):
            issue_step(kv_group(g + 1), t)

        @pl.when(g + 2 < last)
        def _():
            for t in range(2):
                issue_step(kv_group(g + 2), t)
        return carry

    lax.fori_loop(0, last - 1, group_step, 0)

    half = [kv_half(last, i) for i in range(2)]
    ending = [lambda t=t: issue_step(half[t // 4], t % 4) for t in range(8)]
    ending += [lambda t=t: issue_tail(t) for t in range(_WS)]
    arrived = {1: (kv_group(last - 1), (last - 1) * _G), 5: (half[0], last * _G),
               9: (half[1], last * _G + _G // 2)}
    for i, start in enumerate(ending):
        start()
        if i in arrived:
            grp, pair = arrived[i]
            wait_group(grp)
            todo += range(pair, pair + grp[0][0].shape[0], 2)
        if todo:
            attend_two(todo.pop(0))
    assert not todo

    for i in range(_HS):
        project(i)


@jax.jit
def pallas_concat_heads__compressed_kv_cla__mha_block_cached__decode_kernel(
    A_x: jax.Array,
    A_c_kv: jax.Array,
    A_w_q: jax.Array,
    A_w_uk: jax.Array,
    A_w_uv: jax.Array,
    A_w_o: jax.Array,
    B_x: jax.Array,
    B_k_cache: jax.Array,
    B_v_cache: jax.Array,
    B_wq: jax.Array,
    B_wo: jax.Array,
):
    assert A_x.shape == (_B, 1, _M) and A_c_kv.shape == (_B, _SK, _DC)
    assert A_w_q.shape == (_M, _H, _D) and B_k_cache.shape == (_B, _H, _SK, _D)

    up = (_WS, _SLAB // (_H * _D), _H, _D)
    tall = (_WS, _SLAB // _M, _M)
    wide = (_WS, _SLAB // (_H * _D), _H * _D)
    ckv = (2, 8, _SLAB // _DC, _DC)
    kv = (_B * _H // _G, _G, _SK, _D)

    out = pl.pallas_call(
        _kernel,
        in_specs=[pl.BlockSpec(memory_space=pl.ANY)] * 11,
        out_specs=pl.BlockSpec(memory_space=pltpu.VMEM),
        out_shape=jax.ShapeDtypeStruct((_B, 2 * _M), A_x.dtype),
        scratch_shapes=[
            pltpu.VMEM((_B, _M), _BF16),
            pltpu.VMEM((_B, _M), _BF16),
            pltpu.VMEM(ckv, _BF16),
            pltpu.VMEM(up, _BF16),
            pltpu.VMEM(up, _BF16),
            pltpu.VMEM(up, _BF16),
            pltpu.VMEM(tall, _BF16),
            pltpu.VMEM(wide, _BF16),
            pltpu.VMEM(tall, _BF16),
            pltpu.VMEM((_SLOTS, 2) + kv[1:], _BF16),
            pltpu.VMEM((128, 128 * _HG), _BF16),
            pltpu.VMEM((_H, 8, _D), _F32),
            pltpu.VMEM((_H, 8, _D), _F32),
            pltpu.VMEM((_H, 8, _D), _F32),
            pltpu.VMEM((8, 2 * _M), _F32),
            pltpu.SemaphoreType.DMA((2,)),
            pltpu.SemaphoreType.DMA((6,)),
            pltpu.SemaphoreType.DMA((2 * _SLOTS,)),
            pltpu.SemaphoreType.DMA((4,)),
            pltpu.SemaphoreType.DMA((2 * _HS,)),
        ],
        compiler_params=pltpu.CompilerParams(vmem_limit_bytes=100 * 1024 * 1024),
    )(A_x.reshape(_B, _M), A_c_kv.reshape(ckv), A_w_q.reshape(up), A_w_uk.reshape(up),
      A_w_uv.reshape(up), A_w_o.reshape(tall), B_x.reshape(_B, _M), B_k_cache.reshape(kv),
      B_v_cache.reshape(kv), B_wq.reshape(wide), B_wo.reshape(tall))
    return out.reshape(_B, 1, 2 * _M)
```
